```python
import os as _os
_os.environ.setdefault("JAX_PLATFORMS", "cpu")
import jax
import jax.numpy as jnp

def _softmax(x, axis=-1):
    return jax.nn.softmax(x, axis=axis)
def _gelu(x):
    return jax.nn.gelu(x, approximate=True)
def _silu(x):
    return jax.nn.silu(x)
def _sigmoid(x):
    return jax.nn.sigmoid(x)
def _layernorm(x, axis=-1, eps=1e-5):
    m = jnp.mean(x, axis=axis, keepdims=True)
    v = jnp.var(x, axis=axis, keepdims=True)
    return (x - m) / jnp.sqrt(v + eps)
def _scatter_add(tgt, idx, src, axis=0):
    return tgt.at[idx].add(src)
def _segment_sum(src, seg, n):
    return jax.ops.segment_sum(src, seg, n)
class _Rng:
    def __init__(self, key):
        self._k = key
    def _next(self):
        self._k, sub = jax.random.split(self._k)
        return sub
    def normal(self, shape):
        return jax.random.normal(self._next(), shape, dtype=jnp.bfloat16)
    def randint(self, lo, hi, shape):
        return jax.random.randint(self._next(), shape, lo, hi, dtype=jnp.int32)
    def uniform(self, shape, lo=0.0, hi=1.0):
        return jax.random.uniform(self._next(), shape, jnp.bfloat16, lo, hi)
    def permutation(self, n):
        return jax.random.permutation(self._next(), n)


kernel_name = 'concat_heads__sliding_block_cached__sliding_block_cached__decode'

def setup_inputs():
    _rng = _Rng(jax.random.key(int.from_bytes(__import__("os").urandom(4), "little")))
    _w = (lambda a: (lambda t: t.astype(jnp.bfloat16) if jnp.issubdtype(t.dtype, jnp.floating) else t)(jnp.asarray(a)))
    def _A_setup():
        B, Sq, D = 4, 1, 576
        Hq, Hkv, Sk, Dh = 32, 16, 8192, 128
        assert Hq % Hkv == 0, (Hq, Hkv)
        return {
            "x": _w((lambda *s: _rng.normal(s) * 0.8)(B, Sq, D)),
            "k_cache": _w((lambda *s: _rng.normal(s) * 0.8)(B, Hkv, Sk, Dh)),
            "v_cache": _w((lambda *s: _rng.normal(s) * 0.05)(B, Hkv, Sk, Dh)),
            "wq": _w((lambda *s: _rng.normal(s) * 0.8)(D, Hq * Dh) * (D ** -0.5)),
            "wo": _w((lambda *s: _rng.normal(s) * 0.05)(Hq * Dh, D) * ((Hq * Dh) ** -0.5)),
        }
    _A_in = _A_setup()

    def _B_setup():
        B, Sq, D = 4, 1, 576
        Hq, Hkv, Sk, Dh = 32, 16, 8192, 128
        assert Hq % Hkv == 0, (Hq, Hkv)
        return {
            "x": _w((lambda *s: _rng.normal(s) * 0.8)(B, Sq, D)),
            "k_cache": _w((lambda *s: _rng.normal(s) * 0.8)(B, Hkv, Sk, Dh)),
            "v_cache": _w((lambda *s: _rng.normal(s) * 0.05)(B, Hkv, Sk, Dh)),
            "wq": _w((lambda *s: _rng.normal(s) * 0.8)(D, Hq * Dh) * (D ** -0.5)),
            "wo": _w((lambda *s: _rng.normal(s) * 0.05)(Hq * Dh, D) * ((Hq * Dh) ** -0.5)),
        }
    _B_in = _B_setup()

    return {
        "A_x": _A_in["x"],
        "A_k_cache": _A_in["k_cache"],
        "A_v_cache": _A_in["v_cache"],
        "A_wq": _A_in["wq"],
        "A_wo": _A_in["wo"],
        "B_x": _B_in["x"],
        "B_k_cache": _B_in["k_cache"],
        "B_v_cache": _B_in["v_cache"],
        "B_wq": _B_in["wq"],
        "B_wo": _B_in["wo"],
    }

def reference(A_x, A_k_cache, A_v_cache, A_wq, A_wo, B_x, B_k_cache, B_v_cache, B_wq, B_wo):
    def _A_ref(x, k_cache, v_cache, wq, wo):
        B, Sq, D = x.shape
        Hq, Dh = 32, 128
        Hkv, Sk = k_cache.shape[1], k_cache.shape[2]
        W = min(4096, max(256, Sk // 4))
        rep = Hq // Hkv
        q = (lambda x, *d: x.transpose(*d))((x @ wq).reshape(B, Sq, Hq, Dh), 0, 2, 1, 3)
        k = jnp.repeat(k_cache[:, :, Sk - W:, :], rep, axis=1)
        v = jnp.repeat(v_cache[:, :, Sk - W:, :], rep, axis=1)
        scores = jnp.einsum("bhqd,bhkd->bhqk", q, k) * (Dh ** -0.5)
        p = _softmax(scores, axis=-1)
        o = jnp.einsum("bhqk,bhkd->bhqd", p, v)
        return (lambda x, *d: x.transpose(*d))(o, 0, 2, 1, 3).reshape(B, Sq, Hq * Dh) @ wo

    def _B_ref(x, k_cache, v_cache, wq, wo):
        B, Sq, D = x.shape
        Hq, Dh = 32, 128
        Hkv, Sk = k_cache.shape[1], k_cache.shape[2]
        W = min(4096, max(256, Sk // 4))
        rep = Hq // Hkv
        q = (lambda x, *d: x.transpose(*d))((x @ wq).reshape(B, Sq, Hq, Dh), 0, 2, 1, 3)
        k = jnp.repeat(k_cache[:, :, Sk - W:, :], rep, axis=1)
        v = jnp.repeat(v_cache[:, :, Sk - W:, :], rep, axis=1)
        scores = jnp.einsum("bhqd,bhkd->bhqk", q, k) * (Dh ** -0.5)
        p = _softmax(scores, axis=-1)
        o = jnp.einsum("bhqk,bhkd->bhqd", p, v)
        return (lambda x, *d: x.transpose(*d))(o, 0, 2, 1, 3).reshape(B, Sq, Hq * Dh) @ wo

    a = _A_ref(A_x, A_k_cache, A_v_cache, A_wq, A_wo)
    b = _B_ref(B_x, B_k_cache, B_v_cache, B_wq, B_wo)
    return jnp.concatenate([a, b], axis=-1)
```

```python
import functools
import jax
import jax.numpy as jnp
from jax import lax
from jax.experimental import pallas as pl
from jax.experimental.pallas import tpu as pltpu

_NT = (((1,), (1,)), ((), ()))
_NN = (((1,), (0,)), ((), ()))


def _pieces(total, sizes):
    out, off, i = [], 0, 0
    while off < total:
        s = min(sizes[i % len(sizes)], total - off)
        out.append((off, s))
        off += s
        i += 1
    return out


def _deal(items, n):
    return [items[(len(items) * i) // n:(len(items) * (i + 1)) // n] for i in range(n)]


def make(sizes=(96,), order='skb', G=128, wsizes=(640,), worder='spread', nbuf=3, cp=None, OG=4, wo_split=(3, 6)):
    def fn(A_x, A_k, A_v, A_wq, A_wo, B_x, B_k, B_v, B_wq, B_wo):
        B, Sq, D = A_x.shape
        _, Hkv, Sk, Dh = A_k.shape
        Hq = 32
        W = min(4096, max(256, Sk // 4))
        HD = Hq * Dh
        T = 2 * Hkv
        scale = Dh ** -0.5
        NCH = (2 * D) // 128
        NG = W // G
        LA = nbuf - 1
        f32, bf16 = jnp.float32, jnp.bfloat16
        P = _pieces(W, sizes)
        if order == 'skb':
            plan = [(i, b, o, s) for (o, s) in P for i in range(2) for b in range(B)]
        elif order == 'ksb':
            plan = [(i, b, o, s) for i in range(2) for (o, s) in P for b in range(B)]
        plan = [x + (n % 2,) for n, x in enumerate(plan)]
        WP = _pieces(HD, wsizes)

        def kernel(ax, ak, av, awq, awo, bx, bk, bv, bwq, bwo, out_ref,
                   xbuf, wqbuf, wobuf, kvbuf, o_scr, xsem, wqsem, wosem, kvsem):
            def start_kv(k, v, j, slot, items):
                for (i, b, o, s, p) in items:
                    pltpu.make_async_copy(
                        (k, v)[i].at[b, j, pl.ds(Sk - W + o, s), :],
                        kvbuf.at[slot, i, b, pl.ds(o, s), :],
                        kvsem.at[slot]).start(priority=p)

            def wo_items(c):
                rows = list(range(128 * c, 128 * (c + 1), 16))
                if worder == 'spread':
                    return [(c, r, o, s) for (o, s) in WP for r in rows]
                return [(c, r, o, s) for r in rows for (o, s) in WP]

            wo_plan = [x for c in range(NCH) for x in wo_items(c)]
            wo_plan = [x + (n % 2,) for n, x in enumerate(wo_plan)]

            def start_wo(items):
                for (c, r, o, s, p) in items:
                    src = awo.at[pl.ds(r, 16), pl.ds(o, s)] if r < D else bwo.at[pl.ds(r - D, 16), pl.ds(o, s)]
                    pltpu.make_async_copy(src, wobuf.at[pl.ds(r, 16), pl.ds(o, s)], wosem.at[c]).start(priority=p)

            xc = [pltpu.make_async_copy(ax, xbuf.at[0], xsem.at[0]),
                  pltpu.make_async_copy(bx, xbuf.at[1], xsem.at[1])]

            def wq_body(r, c):
                n = 0
                for (o, s) in WP:
                    for g in range(4):
                        r0 = pl.multiple_of(r * 16 + g * (D // 4), 16)
                        for h, w in enumerate((awq, bwq)):
                            pltpu.make_async_copy(w.at[pl.ds(r0, 16), pl.ds(o, s)],
                                                  wqbuf.at[h, pl.ds(r0, 16), pl.ds(o, s)],
                                                  wqsem.at[0]).start(priority=n % 2)
                            n += 1
                return c
            xc[0].start()
            xc[1].start()
            lax.fori_loop(0, D // 64, wq_body, 0)

            def pro(t, c):
                start_kv(ak, av, t, t, plan)
                return c
            lax.fori_loop(0, LA, pro, 0)
            xc[0].wait()
            xc[1].wait()
            pltpu.make_async_copy(wqbuf, wqbuf, wqsem.at[0]).wait()

            row = lax.broadcasted_iota(jnp.int32, (8, Dh), 0)
            rowg = lax.broadcasted_iota(jnp.int32, (8, G), 0) % B
            rowd = row % B
            kv_groups = _deal(plan, 2 * NG)
            per_chunk = len(wo_plan) // NCH
            cuts = [0] + [c * per_chunk for c in wo_split]
            wo_groups = [_deal(wo_plan[cuts[i]:cuts[i + 1]], 2 * NG) for i in range(len(wo_split))]

            def step(t, c):
                slot = lax.rem(t, nbuf)
                tn = t + LA
                nslot = lax.rem(tn, nbuf)
                h = t // Hkv
                j = t - h * Hkv

                def issue(i):
                    @pl.when(tn < Hkv)
                    def _():
                        start_kv(ak, av, tn, nslot, kv_groups[i])

                    @pl.when(jnp.logical_and(tn >= Hkv, tn < T))
                    def _():
                        start_kv(bk, bv, tn - Hkv, nslot, kv_groups[i])

                    for n, grp in enumerate(wo_groups):
                        @pl.when(tn == T + n)
                        def _():
                            start_wo(grp[i])

                x4 = xbuf[h].astype(f32)
                x8 = jnp.concatenate([x4, x4], axis=0).astype(bf16)
                off = pl.multiple_of(j * 2 * Dh, 2 * Dh)
                q2 = lax.dot_general(x8, wqbuf[h, :, pl.ds(off, 2 * Dh)], _NN, preferred_element_type=f32)
                q = jnp.where(row < B, q2[:, :Dh], q2[:, Dh:]).astype(bf16)

                pltpu.make_async_copy(kvbuf.at[slot], kvbuf.at[slot], kvsem.at[slot]).wait()
                ss = []
                for g in range(NG):
                    s = None
                    for b in range(B):
                        sb = lax.dot_general(q, kvbuf[slot, 0, b, pl.ds(g * G, G), :], _NT, preferred_element_type=f32)
                        s = sb if s is None else jnp.where(rowg == b, sb, s)
                    ss.append(s * scale)
                    issue(g)
                m = functools.reduce(jnp.maximum, ss)
                m = jnp.max(m, axis=-1, keepdims=True)
                lacc = None
                acc = [None] * B
                for g in range(NG):
                    p = jnp.exp(ss[g] - m)
                    lacc = p if lacc is None else lacc + p
                    pb = p.astype(bf16)
                    for b in range(B):
                        ob = lax.dot_general(pb, kvbuf[slot, 1, b, pl.ds(g * G, G), :], _NN, preferred_element_type=f32)
                        acc[b] = ob if acc[b] is None else acc[b] + ob
                    issue(NG + g)
                l = jnp.sum(lacc, axis=-1, keepdims=True)
                o = acc[0]
                for b in range(1, B):
                    o = jnp.where(rowd == b, acc[b], o)
                o_scr[t] = o / l
                return c

            lax.fori_loop(0, T, step, 0)

            cols = []
            for j in range(Hkv):
                a = o_scr[j]
                b_ = o_scr[Hkv + j]
                cols.append(jnp.where(row < B, a, pltpu.roll(b_, B, 0)).astype(bf16))
                cols.append(jnp.where(row < B, pltpu.roll(a, B, 0), b_).astype(bf16))
            lane = lax.broadcasted_iota(jnp.int32, (B, 128), 1)
            nog = Hq // OG
            rest = _deal(wo_plan[cuts[-1]:], wo_split[-1] * nog)
            for ci in range(NCH):
                lo = 128 * ci
                blk = wobuf.at[pl.ds(lo, 128), :]
                pltpu.make_async_copy(blk, blk, wosem.at[ci]).wait()
                r = None
                for g in range(nog):
                    lhs = jnp.concatenate(cols[g * OG:(g + 1) * OG], axis=1)
                    rg = lax.dot_general(lhs, wobuf[pl.ds(lo, 128), pl.ds(g * OG * Dh, OG * Dh)], _NT,
                                         preferred_element_type=f32)
                    r = rg if r is None else r + rg
                    if ci * nog + g < len(rest):
                        start_wo(rest[ci * nog + g])
                if lo + 128 <= D:
                    res = r[:B]
                elif lo >= D:
                    res = r[B:]
                else:
                    res = jnp.where(lane < D - lo, r[:B], r[B:])
                out_ref[:, pl.ds(lo, 128)] = res.astype(out_ref.dtype)

        anyspec = pl.BlockSpec(memory_space=pl.ANY)
        out = pl.pallas_call(
            kernel,
            out_shape=jax.ShapeDtypeStruct((B, 2 * D), A_x.dtype),
            in_specs=[anyspec] * 10,
            scratch_shapes=[
                pltpu.VMEM((2, B, D), bf16),
                pltpu.VMEM((2, D, HD), bf16),
                pltpu.VMEM((2 * D, HD), bf16),
                pltpu.VMEM((nbuf, 2, B, W, Dh), bf16),
                pltpu.VMEM((T, 8, Dh), f32),
                pltpu.SemaphoreType.DMA((2,)),
                pltpu.SemaphoreType.DMA((1,)),
                pltpu.SemaphoreType.DMA((NCH,)),
                pltpu.SemaphoreType.DMA((nbuf,)),
            ],
            compiler_params=pltpu.CompilerParams(vmem_limit_bytes=100 * 1024 * 1024, **(cp or {})),
        )(A_x.reshape(B, D), A_k, A_v, A_wq, A_wo.T, B_x.reshape(B, D), B_k, B_v, B_wq, B_wo.T)
        return out.reshape(B, Sq, 2 * D)
    return fn


_impl = make(**dict(cp=dict(disable_bounds_checks=True)))


@jax.jit
def pallas_concat_heads__sliding_block_cached__sliding_block_cached__decode_kernel(
    A_x, A_k_cache, A_v_cache, A_wq, A_wo, B_x, B_k_cache, B_v_cache, B_wq, B_wo,
):
    return _impl(A_x, A_k_cache, A_v_cache, A_wq, A_wo, B_x, B_k_cache, B_v_cache, B_wq, B_wo)
```

```python
import jax
import jax.numpy as jnp
from jax import lax
import jax.experimental.pallas as pl
import jax.experimental.pallas.tpu as pltpu

_NN = (((1,), (0,)), ((), ()))
_NT = (((1,), (1,)), ((), ()))

_HQ = 32
_LANES = 128
_NBUF = 3
_AHEAD = _NBUF - 1
_KV_ROWS = (64, 128)
_W_ROWS = 8
_W_COLS = (1024, 2048, 1024)


def _spans(sizes):
    return [(sum(sizes[:i]), s) for i, s in enumerate(sizes)]


def _wo_copy_plan(n_rows, n_cols):
    half = n_cols // 2
    last = n_rows - _LANES
    parts = [
        (0, last - 2 * _LANES, 0, n_cols),
        (last - 2 * _LANES, _LANES, 0, n_cols),
        (last - _LANES, _LANES, 0, n_cols),
        (last, _LANES, 0, half),
        (last, _LANES, half, half),
    ]

    def copies(part, streams, cols, queue):
        per = parts[part][1] // streams
        return [
            (part, i * per + r, c, n, queue(i))
            for r in range(0, per, _W_ROWS)
            for (c, n) in _spans(cols)
            for i in range(streams)
        ]

    bulk = copies(0, 8, _W_COLS, lambda i: i % 2)
    third = len(bulk) // 3
    in_loop = [
        bulk[:third],
        bulk[third : 2 * third],
        bulk[2 * third :],
        copies(1, 4, _W_COLS, lambda i: i % 2),
    ]
    first = copies(2, 4, (half, half), lambda i: 0)
    second = copies(3, 4, (half,), lambda i: 1) + copies(4, 4, (half,), lambda i: 1)
    final = [c for pair in zip(first, second) for c in pair]
    return parts, in_loop, final


@jax.jit
def pallas_concat_heads__sliding_block_cached__sliding_block_cached__decode_kernel(
    A_x: jax.Array,
    A_k_cache: jax.Array,
    A_v_cache: jax.Array,
    A_wq: jax.Array,
    A_wo: jax.Array,
    B_x: jax.Array,
    B_k_cache: jax.Array,
    B_v_cache: jax.Array,
    B_wq: jax.Array,
    B_wo: jax.Array,
):
    B, Sq, D = A_x.shape
    _, Hkv, Sk, Dh = A_k_cache.shape
    W = min(4096, max(256, Sk // 4))
    HD = _HQ * Dh
    R = 2 * B
    T = 2 * Hkv
    assert (B, Sq, Dh, _HQ) == (4, 1, _LANES, 2 * Hkv) and sum(_W_COLS) == HD
    assert D % (4 * _W_ROWS) == 0 and (2 * D) % _LANES == 0 and W % 16 == 0
    scale = Dh**-0.5
    f32, bf16 = jnp.float32, jnp.bfloat16

    period = sum(_KV_ROWS)
    n_periods = W // period
    wo_parts, wo_in_loop, wo_final = _wo_copy_plan(2 * D, HD)
    wq_sem, x_sem = _AHEAD, _NBUF
    wo_sems = [T % _NBUF, (T + 1) % _NBUF, (T + 2) % _NBUF, _NBUF, T % _NBUF]

    def kernel(ax, ak, av, awq, awo_t, bx, bk, bv, bwq, bwo_t, out_ref,
               x_buf, wq_buf, kv_buf, o_heads, o_cat, acc, sem, *wo_bufs):
        def wait_filled(buf, s):
            pltpu.make_async_copy(buf, buf, sem.at[s]).wait()

        def start_kv_rows(k, v, head, slot, off, n):
            for i, src in enumerate((k, v)):
                for b in range(B):
                    pltpu.make_async_copy(
                        src.at[b, head, pl.ds(Sk - W + off, n), :],
                        kv_buf.at[slot, i, b, pl.ds(off, n), :],
                        sem.at[slot],
                    ).start(priority=b % 2)

        def start_kv(k, v, head, slot, lo, hi):
            def body(r, carry):
                for (off, n) in _spans(_KV_ROWS):
                    start_kv_rows(k, v, head, slot, pl.multiple_of(r * period + off, 16), n)
                return carry

            lax.fori_loop(lo, hi, body, 0)
            if hi == n_periods and W > n_periods * period:
                start_kv_rows(k, v, head, slot, n_periods * period, W - n_periods * period)

        def start_wo(copies):
            for (part, r, c, n, queue) in copies:
                row, col = wo_parts[part][0] + r, wo_parts[part][2] + c
                src, row = (awo_t, row) if row < D else (bwo_t, row - D)
                pltpu.make_async_copy(
                    src.at[pl.ds(row, _W_ROWS), pl.ds(col, n)],
                    wo_bufs[part].at[pl.ds(r, _W_ROWS), pl.ds(c, n)],
                    sem.at[wo_sems[part]],
                ).start(priority=queue)

        def start_wq(r, carry):
            for (c, n) in _spans(_W_COLS):
                for h, src in enumerate((awq, bwq)):
                    for i in range(4):
                        row = pl.multiple_of(r * _W_ROWS + i * (D // 4), _W_ROWS)
                        pltpu.make_async_copy(
                            src.at[pl.ds(row, _W_ROWS), pl.ds(c, n)],
                            wq_buf.at[h, pl.ds(row, _W_ROWS), pl.ds(c, n)],
                            sem.at[wq_sem],
                        ).start(priority=i % 2)
            return carry

        lax.fori_loop(0, D // (4 * _W_ROWS), start_wq, 0)
        x_copies = [
            pltpu.make_async_copy(src, x_buf.at[h], sem.at[x_sem])
            for h, src in enumerate((ax, bx))
        ]
        for copy in x_copies:
            copy.start()

        def start_first_kv(t, carry):
            start_kv(ak, av, t, t, 0, n_periods)
            return carry

        lax.fori_loop(0, _AHEAD, start_first_kv, 0)
        wait_filled(wq_buf, wq_sem)
        for copy in x_copies:
            copy.wait()

        row_id = lax.broadcasted_iota(jnp.int32, (R, Dh), 0)
        top = row_id < B
        batch_of_row = row_id % B
        batch_of_row_w = lax.broadcasted_iota(jnp.int32, (R, W), 0) % B

        def step(t, carry):
            slot = lax.rem(t, _NBUF)
            h = t // Hkv
            head = t - h * Hkv
            nxt = t + _AHEAD
            nxt_slot = lax.rem(nxt, _NBUF)

            def feed_stream(i):
                lo, hi = ((0, n_periods // 2), (n_periods // 2, n_periods))[i]

                @pl.when(nxt < Hkv)
                def _():
                    start_kv(ak, av, nxt, nxt_slot, lo, hi)

                @pl.when(jnp.logical_and(nxt >= Hkv, nxt < T))
                def _():
                    start_kv(bk, bv, nxt - Hkv, nxt_slot, lo, hi)

                for n in range(_AHEAD):

                    @pl.when(nxt == T + n)
                    def _():
                        start_wo(wo_in_loop[2 * n + i])

            x = x_buf[h].astype(f32)
            x = jnp.concatenate([x, x], axis=0).astype(bf16)
            col = pl.multiple_of(head * 2 * Dh, 2 * Dh)
            q = lax.dot_general(
                x, wq_buf[h, :, pl.ds(col, 2 * Dh)], _NN, preferred_element_type=f32
            )
            q = jnp.where(top, q[:, :Dh], q[:, Dh:]).astype(bf16)

            wait_filled(kv_buf.at[slot], slot)

            s = None
            for b in range(B):
                s_b = lax.dot_general(q, kv_buf[slot, 0, b], _NT, preferred_element_type=f32)
                s = s_b if s is None else jnp.where(batch_of_row_w == b, s_b, s)
            s = s * scale
            p = jnp.exp(s - jnp.max(s, axis=-1, keepdims=True))
            denom = jnp.sum(p, axis=-1, keepdims=True)
            p = p.astype(bf16)
            feed_stream(0)

            o = None
            for b in range(B):
                o_b = lax.dot_general(p, kv_buf[slot, 1, b], _NN, preferred_element_type=f32)
                o = o_b if o is None else jnp.where(batch_of_row == b, o_b, o)
            o_heads[t] = o / denom
            feed_stream(1)
            return carry

        lax.fori_loop(0, T, step, 0)

        for j in range(Hkv):
            o_a, o_b = o_heads[j], o_heads[Hkv + j]
            even = jnp.where(top, o_b, pltpu.roll(o_a, B, 0))
            odd = jnp.where(top, pltpu.roll(o_b, B, 0), o_a)
            o_cat[:, pl.ds(2 * j * Dh, Dh)] = even.astype(bf16)
            o_cat[:, pl.ds((2 * j + 1) * Dh, Dh)] = odd.astype(bf16)

        def project(part, r=0):
            _, _, col, n = wo_parts[part]
            return lax.dot_general(
                o_cat[:, pl.ds(col, n)], wo_bufs[part][pl.ds(r, _LANES), :], _NT,
                preferred_element_type=f32,
            )

        def emit(col, res):
            if col + _LANES <= D:
                res = res[B:]
            elif col >= D:
                res = res[:B]
            else:
                lane = lax.broadcasted_iota(jnp.int32, (B, _LANES), 1)
                res = jnp.where(lane < D - col, res[B:], res[:B])
            out_ref[:, pl.ds(col, _LANES)] = res.astype(out_ref.dtype)

        wait_filled(wo_bufs[0], wo_sems[0])
        half = len(wo_final) // 2
        for n, r in enumerate(range(0, wo_parts[0][1], _LANES)):
            emit(r, project(0, r))
            if n == 1:
                start_wo(wo_final[:half])
            elif n == 2:
                start_wo(wo_final[half:])
        wait_filled(wo_bufs[1], wo_sems[1])
        emit(wo_parts[1][0], project(1))
        wait_filled(wo_bufs[3], wo_sems[3])
        acc[...] = project(3)
        wait_filled(wo_bufs[2], wo_sems[2])
        emit(wo_parts[2][0], project(2))
        wait_filled(wo_bufs[4], wo_sems[4])
        emit(wo_parts[4][0], acc[...] + project(4))

    out = pl.pallas_call(
        kernel,
        out_shape=jax.ShapeDtypeStruct((B, 2 * D), A_x.dtype),
        in_specs=[pl.BlockSpec(memory_space=pl.ANY)] * 10,
        scratch_shapes=[
            pltpu.VMEM((2, B, D), bf16),
            pltpu.VMEM((2, D, HD), bf16),
            pltpu.VMEM((_NBUF, 2, B, W, Dh), bf16),
            pltpu.VMEM((T, R, Dh), f32),
            pltpu.VMEM((R, HD), bf16),
            pltpu.VMEM((R, _LANES), f32),
            pltpu.SemaphoreType.DMA((_NBUF + 1,)),
        ]
        + [pltpu.VMEM((rows, cols), bf16) for (_, rows, _, cols) in wo_parts],
        compiler_params=pltpu.CompilerParams(vmem_limit_bytes=64 * 1024 * 1024),
    )(
        A_x.reshape(B, D), A_k_cache, A_v_cache, A_wq, A_wo.T,
        B_x.reshape(B, D), B_k_cache, B_v_cache, B_wq, B_wo.T,
    )
    return out.reshape(B, Sq, 2 * D)
```

```python
import jax
import jax.numpy as jnp
from jax import lax
import jax.experimental.pallas as pl
import jax.experimental.pallas.tpu as pltpu

_NN = (((1,), (0,)), ((), ()))
_NT = (((1,), (1,)), ((), ()))

_HQ = 32
_LANES = 128
_NBUF = 3
_AHEAD = _NBUF - 1
_KV_ROWS = (64, 128)
_HEAD_SHIFT = (0, 4, 8, 12)
_W_ROWS = 8
_W_COLS = (1024, 2048, 1024)


def _spans(sizes):
    return [(sum(sizes[:i]), s) for i, s in enumerate(sizes)]


def _wo_copy_plan(n_rows, n_cols):
    half = n_cols // 2
    last = n_rows - _LANES
    parts = [
        (0, last - 2 * _LANES, 0, n_cols),
        (last - 2 * _LANES, _LANES, 0, n_cols),
        (last - _LANES, _LANES, 0, n_cols),
        (last, _LANES, 0, half),
        (last, _LANES, half, half),
    ]

    def copies(part, streams, cols, queue):
        per = parts[part][1] // streams
        return [
            (part, i * per + r, c, n, queue(i))
            for r in range(0, per, _W_ROWS)
            for (c, n) in _spans(cols)
            for i in range(streams)
        ]

    bulk = copies(0, 8, _W_COLS, lambda i: i % 2)
    third = len(bulk) // 3
    in_loop = [
        bulk[:third],
        bulk[third : 2 * third],
        bulk[2 * third :],
        copies(1, 4, _W_COLS, lambda i: i % 2),
    ]
    first = copies(2, 4, (half, half), lambda i: 0)
    second = copies(3, 4, (half,), lambda i: 1) + copies(4, 4, (half,), lambda i: 1)
    final = [c for pair in zip(first, second) for c in pair]
    return parts, in_loop, final


@jax.jit
def pallas_concat_heads__sliding_block_cached__sliding_block_cached__decode_kernel(
    A_x: jax.Array,
    A_k_cache: jax.Array,
    A_v_cache: jax.Array,
    A_wq: jax.Array,
    A_wo: jax.Array,
    B_x: jax.Array,
    B_k_cache: jax.Array,
    B_v_cache: jax.Array,
    B_wq: jax.Array,
    B_wo: jax.Array,
):
    B, Sq, D = A_x.shape
    _, Hkv, Sk, Dh = A_k_cache.shape
    W = min(4096, max(256, Sk // 4))
    HD = _HQ * Dh
    R = 2 * B
    T = 2 * Hkv
    assert (B, Sq, Dh, _HQ) == (4, 1, _LANES, 2 * Hkv) and sum(_W_COLS) == HD
    assert D % (4 * _W_ROWS) == 0 and (2 * D) % _LANES == 0 and W % 16 == 0
    scale = Dh**-0.5
    f32, bf16 = jnp.float32, jnp.bfloat16

    period = sum(_KV_ROWS)
    n_periods = W // period
    wo_parts, wo_in_loop, wo_final = _wo_copy_plan(2 * D, HD)
    wq_sem, x_sem = _AHEAD, _NBUF
    wo_sems = [T % _NBUF, (T + 1) % _NBUF, (T + 2) % _NBUF, _NBUF, T % _NBUF]

    def kernel(ax, ak, av, awq, awo_t, bx, bk, bv, bwq, bwo_t, out_ref,
               x_buf, wq_buf, kv_buf, o_steps, o_cat, acc, sem, *wo_bufs):
        def wait_filled(buf, s):
            pltpu.make_async_copy(buf, buf, sem.at[s]).wait()

        def start_kv_rows(k, v, heads, slot, off, n):
            for i, src in enumerate((k, v)):
                for b in range(B):
                    pltpu.make_async_copy(
                        src.at[b, heads[b], pl.ds(Sk - W + off, n), :],
                        kv_buf.at[slot, i, b, pl.ds(off, n), :],
                        sem.at[slot],
                    ).start(priority=b % 2)

        def start_kv(k, v, j, slot, lo, hi):
            heads = [lax.rem(j + shift, Hkv) for shift in _HEAD_SHIFT]

            def body(r, carry):
                for (off, n) in _spans(_KV_ROWS):
                    start_kv_rows(k, v, heads, slot, pl.multiple_of(r * period + off, 16), n)
                return carry

            lax.fori_loop(lo, hi, body, 0)
            if hi == n_periods and W > n_periods * period:
                start_kv_rows(k, v, heads, slot, n_periods * period, W - n_periods * period)

        def start_wo(copies):
            for (part, r, c, n, queue) in copies:
                row, col = wo_parts[part][0] + r, wo_parts[part][2] + c
                src, row = (awo_t, row) if row < D else (bwo_t, row - D)
                pltpu.make_async_copy(
                    src.at[pl.ds(row, _W_ROWS), pl.ds(col, n)],
                    wo_bufs[part].at[pl.ds(r, _W_ROWS), pl.ds(c, n)],
                    sem.at[wo_sems[part]],
                ).start(priority=queue)

        def start_wq(r, carry):
            for (c, n) in _spans(_W_COLS):
                for h, src in enumerate((awq, bwq)):
                    for i in range(4):
                        row = pl.multiple_of(r * _W_ROWS + i * (D // 4), _W_ROWS)
                        pltpu.make_async_copy(
                            src.at[pl.ds(row, _W_ROWS), pl.ds(c, n)],
                            wq_buf.at[h, pl.ds(row, _W_ROWS), pl.ds(c, n)],
                            sem.at[wq_sem],
                        ).start(priority=i % 2)
            return carry

        lax.fori_loop(0, D // (4 * _W_ROWS), start_wq, 0)
        x_copies = [
            pltpu.make_async_copy(src, x_buf.at[h], sem.at[x_sem])
            for h, src in enumerate((ax, bx))
        ]
        for copy in x_copies:
            copy.start()

        def start_first_kv(t, carry):
            start_kv(ak, av, t, t, 0, n_periods)
            return carry

        lax.fori_loop(0, _AHEAD, start_first_kv, 0)
        wait_filled(wq_buf, wq_sem)
        for copy in x_copies:
            copy.wait()

        row_id = lax.broadcasted_iota(jnp.int32, (R, Dh), 0)
        top = row_id < B
        batch_of_row = row_id % B
        batch_of_row_w = lax.broadcasted_iota(jnp.int32, (R, W), 0) % B

        def per_shift(f):
            vals = {shift: f(shift) for shift in sorted(set(_HEAD_SHIFT))}
            res = vals[_HEAD_SHIFT[0]]
            for b in range(1, B):
                if _HEAD_SHIFT[b] != _HEAD_SHIFT[0]:
                    res = jnp.where(batch_of_row == b, vals[_HEAD_SHIFT[b]], res)
            return res

        def step(t, carry):
            slot = lax.rem(t, _NBUF)
            h = t // Hkv
            j = t - h * Hkv
            nxt = t + _AHEAD
            nxt_slot = lax.rem(nxt, _NBUF)

            def feed_stream(i):
                lo, hi = ((0, n_periods // 2), (n_periods // 2, n_periods))[i]

                @pl.when(nxt < Hkv)
                def _():
                    start_kv(ak, av, nxt, nxt_slot, lo, hi)

                @pl.when(jnp.logical_and(nxt >= Hkv, nxt < T))
                def _():
                    start_kv(bk, bv, nxt - Hkv, nxt_slot, lo, hi)

                for n in range(_AHEAD):

                    @pl.when(nxt == T + n)
                    def _():
                        start_wo(wo_in_loop[2 * n + i])

            x = x_buf[h].astype(f32)
            x = jnp.concatenate([x, x], axis=0).astype(bf16)

            def queries(shift):
                col = pl.multiple_of(lax.rem(j + shift, Hkv) * 2 * Dh, 2 * Dh)
                q2 = lax.dot_general(
                    x, wq_buf[h, :, pl.ds(col, 2 * Dh)], _NN, preferred_element_type=f32
                )
                return jnp.where(top, q2[:, :Dh], q2[:, Dh:])

            q = per_shift(queries).astype(bf16)

            wait_filled(kv_buf.at[slot], slot)

            s = None
            for b in range(B):
                s_b = lax.dot_general(q, kv_buf[slot, 0, b], _NT, preferred_element_type=f32)
                s = s_b if s is None else jnp.where(batch_of_row_w == b, s_b, s)
            s = s * scale
            p = jnp.exp(s - jnp.max(s, axis=-1, keepdims=True))
            denom = jnp.sum(p, axis=-1, keepdims=True)
            p = p.astype(bf16)
            feed_stream(0)

            o = None
            for b in range(B):
                o_b = lax.dot_general(p, kv_buf[slot, 1, b], _NN, preferred_element_type=f32)
                o = o_b if o is None else jnp.where(batch_of_row == b, o_b, o)
            o_steps[t] = o / denom
            feed_stream(1)
            return carry

        lax.fori_loop(0, T, step, 0)

        for j in range(Hkv):
            o_a = per_shift(lambda shift: o_steps[(j - shift) % Hkv])
            o_b = per_shift(lambda shift: o_steps[Hkv + (j - shift) % Hkv])
            even = jnp.where(top, o_b, pltpu.roll(o_a, B, 0))
            odd = jnp.where(top, pltpu.roll(o_b, B, 0), o_a)
            o_cat[:, pl.ds(2 * j * Dh, Dh)] = even.astype(bf16)
            o_cat[:, pl.ds((2 * j + 1) * Dh, Dh)] = odd.astype(bf16)

        def project(part, r=0):
            _, _, col, n = wo_parts[part]
            return lax.dot_general(
                o_cat[:, pl.ds(col, n)], wo_bufs[part][pl.ds(r, _LANES), :], _NT,
                preferred_element_type=f32,
            )

        def emit(col, res):
            if col + _LANES <= D:
                res = res[B:]
            elif col >= D:
                res = res[:B]
            else:
                lane = lax.broadcasted_iota(jnp.int32, (B, _LANES), 1)
                res = jnp.where(lane < D - col, res[B:], res[:B])
            out_ref[:, pl.ds(col, _LANES)] = res.astype(out_ref.dtype)

        wait_filled(wo_bufs[0], wo_sems[0])
        half = len(wo_final) // 2
        for n, r in enumerate(range(0, wo_parts[0][1], _LANES)):
            emit(r, project(0, r))
            if n == 1:
                start_wo(wo_final[:half])
            elif n == 2:
                start_wo(wo_final[half:])
        wait_filled(wo_bufs[1], wo_sems[1])
        emit(wo_parts[1][0], project(1))
        wait_filled(wo_bufs[3], wo_sems[3])
        acc[...] = project(3)
        wait_filled(wo_bufs[2], wo_sems[2])
        emit(wo_parts[2][0], project(2))
        wait_filled(wo_bufs[4], wo_sems[4])
        emit(wo_parts[4][0], acc[...] + project(4))

    out = pl.pallas_call(
        kernel,
        out_shape=jax.ShapeDtypeStruct((B, 2 * D), A_x.dtype),
        in_specs=[pl.BlockSpec(memory_space=pl.ANY)] * 10,
        scratch_shapes=[
            pltpu.VMEM((2, B, D), bf16),
            pltpu.VMEM((2, D, HD), bf16),
            pltpu.VMEM((_NBUF, 2, B, W, Dh), bf16),
            pltpu.VMEM((T, R, Dh), f32),
            pltpu.VMEM((R, HD), bf16),
            pltpu.VMEM((R, _LANES), f32),
            pltpu.SemaphoreType.DMA((_NBUF + 1,)),
        ]
        + [pltpu.VMEM((rows, cols), bf16) for (_, rows, _, cols) in wo_parts],
        compiler_params=pltpu.CompilerParams(vmem_limit_bytes=64 * 1024 * 1024),
    )(
        A_x.reshape(B, D), A_k_cache, A_v_cache, A_wq, A_wo.T,
        B_x.reshape(B, D), B_k_cache, B_v_cache, B_wq, B_wo.T,
    )
    return out.reshape(B, Sq, 2 * D)
```
